```python
import jax
import jax.numpy as jnp

def _softmax(x, axis=-1):
    return jax.nn.softmax(x, axis=axis)

def _gelu(x):
    return jax.nn.gelu(x, approximate=True)

def _silu(x):
    return jax.nn.silu(x)

def _sigmoid(x):
    return jax.nn.sigmoid(x)

def _layernorm(x, axis=-1, eps=1e-05):
    m = jnp.mean(x, axis=axis, keepdims=True)
    v = jnp.var(x, axis=axis, keepdims=True)
    return (x - m) / jnp.sqrt(v + eps)

def _scatter_add(tgt, idx, src, axis=0):
    return tgt.at[idx].add(src)

def _segment_sum(src, seg, n):
    return jax.ops.segment_sum(src, seg, n)

class _Rng:

    def __init__(self, key):
        self._k = key

    def _next(self):
        self._k, sub = jax.random.split(self._k)
        return sub

    def normal(self, shape):
        return jax.random.normal(self._next(), shape, dtype=jnp.bfloat16)

    def randint(self, lo, hi, shape):
        return jax.random.randint(self._next(), shape, lo, hi, dtype=jnp.int32)

    def uniform(self, shape, lo=0.0, hi=1.0):
        return jax.random.uniform(self._next(), shape, jnp.bfloat16, lo, hi)

    def permutation(self, n):
        return jax.random.permutation(self._next(), n)
kernel_name = 'interleave_layers__linear_kernel_hedgehog__memory_aug_recurrent_mem_tr__prompt'

def setup_inputs():
    _rng = _Rng(jax.random.key(int.from_bytes(__import__("os").urandom(4), "little")))
    _w = lambda a: (lambda t: t.astype(jnp.bfloat16) if jnp.issubdtype(t.dtype, jnp.floating) else t)(jnp.asarray(a))

    def _A_setup():
        B, S, D, H = (1, 2048, 640, 32)
        Dh = D // H
        return {'x': _w((lambda *s: _rng.normal(s) * 0.05)(B, S, D)), 'wqkv': _w((lambda *s: _rng.normal(s) * 0.05)(D, 3 * D)), 'w_phi': _w((lambda *s: _rng.normal(s) * 0.05)(H, Dh, Dh) * Dh ** (-0.5)), 'wo': _w((lambda *s: _rng.normal(s) * 0.05)(D, D))}
    _A_in = _A_setup()

    def _B_setup():
        B, S, Dm = (1, 2048, 640)
        H, Dh = (32, 192)
        M, seg = (8, 32)
        seg = min(seg, S)
        S = S // seg * seg
        return {'x': _w((lambda *s: _rng.normal(s) * 0.05)(B, S, Dm)), 'mem0': _w((lambda *s: _rng.normal(s) * 0.05)(B, M, Dm)), 'Wq': _w((lambda *s: _rng.normal(s) * 0.05)(Dm, H, Dh) * Dm ** (-0.5)), 'Wk': _w((lambda *s: _rng.normal(s) * 0.05)(Dm, H, Dh) * Dm ** (-0.5)), 'Wv': _w((lambda *s: _rng.normal(s) * 0.05)(Dm, H, Dh) * Dm ** (-0.5)), 'Wo': _w((lambda *s: _rng.normal(s) * 0.05)(H, Dh, Dm) * (H * Dh) ** (-0.5)), 'seg_len': seg}
    _B_in = _B_setup()
    return {'A_x': _A_in['x'], 'A_wqkv': _A_in['wqkv'], 'A_w_phi': _A_in['w_phi'], 'A_wo': _A_in['wo'], 'B_x': _B_in['x'], 'B_mem0': _B_in['mem0'], 'B_Wq': _B_in['Wq'], 'B_Wk': _B_in['Wk'], 'B_Wv': _B_in['Wv'], 'B_Wo': _B_in['Wo'], 'B_seg_len': _B_in['seg_len']}

def reference(A_x, A_wqkv, A_w_phi, A_wo, B_x, B_mem0, B_Wq, B_Wk, B_Wv, B_Wo, B_seg_len):

    def _A_ref(x, wqkv, w_phi, wo):
        B, S, D = x.shape
        H = 32
        Dh = D // H
        qkv = (lambda x, *d: x.transpose(*d))((x @ wqkv).reshape(B, S, 3, H, Dh), 2, 0, 3, 1, 4)
        q, k, v = (qkv[0], qkv[1], qkv[2])
        pq = jnp.einsum('bhsd,hdf->bhsf', q, w_phi)
        pk = jnp.einsum('bhsd,hdf->bhsf', k, w_phi)
        phi_q = jnp.concatenate([_softmax(pq, axis=-1), _softmax(-pq, axis=-1)], axis=-1)
        phi_k = jnp.concatenate([_softmax(pk, axis=-1), _softmax(-pk, axis=-1)], axis=-1)
        kv = jnp.einsum('bhsf,bhsd->bhfd', phi_k, v)
        z = jnp.einsum('bhsf->bhf', phi_k)
        num = jnp.einsum('bhqf,bhfd->bhqd', phi_q, kv)
        den = jnp.einsum('bhqf,bhf->bhq', phi_q, z)[..., None] + 1e-06
        o = num / den
        return (lambda x, *d: x.transpose(*d))(o, 0, 2, 1, 3).reshape(B, S, D) @ wo

    def _B_ref(x, mem0, Wq, Wk, Wv, Wo, seg_len):
        B, S, Dm = x.shape
        H, Dh = (Wq.shape[1], Wq.shape[2])
        M = mem0.shape[1]
        scale = Dh ** (-0.5)
        n_seg = S // seg_len
        L = M + seg_len
        idx = jnp.arange(L)
        mask = (idx[:, None] < M) | (idx[:, None] >= idx[None, :])
        mem = mem0
        outs = []
        for s in range(n_seg):
            xs = x[:, s * seg_len:(s + 1) * seg_len, :].copy()
            h = jnp.concatenate([mem, xs], axis=1)
            q = jnp.einsum('btd,dhe->bhte', h, Wq)
            k = jnp.einsum('btd,dhe->bhte', h, Wk)
            v = jnp.einsum('btd,dhe->bhte', h, Wv)
            scores = jnp.einsum('bhqe,bhke->bhqk', q, k) * scale
            scores = jnp.where(mask[None, None], scores, -1000000000.0)
            p = _softmax(scores, axis=-1)
            o = jnp.einsum('bhqk,bhke->bhqe', p, v)
            o = jnp.einsum('bhte,hed->btd', o, Wo)
            mem = o[:, :M, :].copy()
            outs.append(o[:, M:, :])
        return jnp.concatenate(outs, axis=1)
    x = A_x
    x = x + _A_ref(_layernorm(x, axis=-1), A_wqkv, A_w_phi, A_wo)
    x = x + _B_ref(_layernorm(x, axis=-1), B_mem0, B_Wq, B_Wk, B_Wv, B_Wo, B_seg_len)
    x = x + _A_ref(_layernorm(x, axis=-1), A_wqkv, A_w_phi, A_wo)
    x = x + _B_ref(_layernorm(x, axis=-1), B_mem0, B_Wq, B_Wk, B_Wv, B_Wo, B_seg_len)
    return x
```

```python
import jax
import jax.numpy as jnp
import jax.experimental.pallas as pl
import jax.experimental.pallas.tpu as pltpu

S, D = 2048, 640
T = 512
SEG, M, L = 32, 8, 40
HD = 6144
F32, BF = jnp.float32, jnp.bfloat16
NT = (((1,), (1,)), ((), ()))
TN = (((0,), (0,)), ((), ()))
WIN = (0, 128, 256, 384)


def _ln(x):
    m = jnp.mean(x, axis=-1, keepdims=True)
    c = x - m
    v = jnp.mean(c * c, axis=-1, keepdims=True)
    return c * jax.lax.rsqrt(v + 1e-5)


def _iota(shape, d):
    return jax.lax.broadcasted_iota(jnp.int32, shape, d)


def _phi(p):
    p = p.reshape(20, 8, p.shape[-1])
    a = jnp.exp(p - jnp.max(p, axis=0, keepdims=True))
    b = jnp.exp(jnp.min(p, axis=0, keepdims=True) - p)
    a = a / jnp.sum(a, axis=0, keepdims=True)
    b = b / jnp.sum(b, axis=0, keepdims=True)
    return a, b


def _kernel(x_ref, wqkv_ref, wp_ref, wo_ref, mem0_ref, wq_h, wk_h, wv_h, wob_h,
            o_ref, xs, lnb, wqt, wkt, kv, zs, wq, wk, wv, wob, mem, sems):
    cps = [pltpu.make_async_copy(s, d, sems.at[i]) for i, (s, d) in
           enumerate(((wq_h, wq), (wk_h, wk), (wv_h, wv), (wob_h, wob)))]
    for c in cps:
        c.start()

    sel = (_iota((128, D), 0) == (_iota((128, D), 1) % 160) // 8).astype(BF)
    bd = jnp.dot(wp_ref[...], sel, preferred_element_type=F32)
    col = _iota((D, D), 1)
    bd = jnp.where(_iota((D, D), 0) // 20 == (col // 160) * 8 + col % 8, bd, 0.0).astype(BF)
    wqt[...] = jnp.dot(wqkv_ref[:, 0:D], bd, preferred_element_type=F32).T.astype(BF)
    wkt[...] = jnp.dot(wqkv_ref[:, D:2 * D], bd, preferred_element_type=F32).T.astype(BF)
    xs[...] = x_ref[...].astype(F32)

    def layer_a():
        kv[...] = jnp.zeros(kv.shape, F32)
        zs[...] = jnp.zeros(zs.shape, F32)

        def pass1(c, _):
            r = pl.ds(pl.multiple_of(c * T, T), T)
            ln = _ln(xs[r, :])
            lnb[r, :] = ln
            ln = ln.astype(BF)
            v = jnp.dot(ln, wqkv_ref[:, 2 * D:3 * D], preferred_element_type=F32).astype(BF)
            for g in range(4):
                p = jax.lax.dot_general(wkt[g * 160:(g + 1) * 160, :], ln, NT,
                                        preferred_element_type=F32)
                a, b = _phi(p)
                ph = jnp.concatenate([a, b], axis=0).reshape(320, T)
                zs[g] += jnp.sum(ph, axis=1, keepdims=True)
                kv[g] += jnp.dot(ph.astype(BF), v[:, WIN[g]:WIN[g] + 256],
                                 preferred_element_type=F32)
            return 0
        jax.lax.fori_loop(0, S // T, pass1, 0)
        for g in range(4):
            own = (_iota((320, 256), 1) + WIN[g]) // 20 == g * 8 + _iota((320, 256), 0) % 8
            kv[g] = jnp.where(own, kv[g], 0.0)

        def pass2(c, _):
            r = pl.ds(pl.multiple_of(c * T, T), T)
            ln = lnb[r, :].astype(BF)
            os = []
            for g in range(4):
                p = jax.lax.dot_general(wqt[g * 160:(g + 1) * 160, :], ln, NT,
                                        preferred_element_type=F32)
                a, b = _phi(p)
                ph = jnp.concatenate([a, b], axis=0)
                den = jnp.sum(ph * zs[g].reshape(40, 8, 1), axis=0, keepdims=True) + 1e-6
                ph = (ph / den).reshape(320, T).astype(BF)
                os.append(jax.lax.dot_general(ph, kv[g].astype(BF), TN,
                                              preferred_element_type=F32))
            o = jnp.concatenate([os[0][:, :128], os[0][:, 128:] + os[1][:, :128],
                                 os[1][:, 128:] + os[2][:, :128],
                                 os[2][:, 128:] + os[3][:, :128], os[3][:, 128:]], axis=1)
            xs[r, :] += jnp.dot(o.astype(BF), wo_ref[...], preferred_element_type=F32)
            return 0
        jax.lax.fori_loop(0, S // T, pass2, 0)

    def layer_b():
        def lnc(c, _):
            r = pl.ds(pl.multiple_of(c * T, T), T)
            lnb[r, :] = _ln(xs[r, :])
            return 0
        jax.lax.fori_loop(0, S // T, lnc, 0)
        mem[...] = mem0_ref[...].astype(F32)

        def step(s, _):
            r = pl.ds(pl.multiple_of(s * SEG, SEG), SEG)
            h = jnp.concatenate([mem[...], lnb[r, :]], axis=0)
            row = _iota((L, 128), 0)
            lane = _iota((L, 128), 1)
            key = lane % 64
            vis = (row < M) | (row >= key)
            head_a = lane < 64
            real = key < L
            first = _iota((L, 384), 1) < 192
            pad = jnp.zeros((64 - L, 384), F32)

            def two(t):
                return jnp.concatenate([jnp.where(first, t, 0.0), pad,
                                        jnp.where(first, 0.0, t), pad], axis=0).astype(BF)

            def proj(p):
                c = slice(p * 384, (p + 1) * 384)
                return [jnp.dot(h, w[:, c], preferred_element_type=F32) for w in (wq, wk, wv)]

            def attn(q, k, v):
                sc = jax.lax.dot_general(q, two(k), NT, preferred_element_type=F32) * (192 ** -0.5)
                sc = jnp.where(vis, sc, -1000000000.0)
                ninf = -jnp.inf
                ma = jnp.max(jnp.where(head_a & real, sc, ninf), axis=1, keepdims=True)
                mb = jnp.max(jnp.where(head_a | ~real, ninf, sc), axis=1, keepdims=True)
                e = jnp.where(real, jnp.exp(sc - jnp.where(head_a, ma, mb)), 0.0)
                sa = jnp.sum(jnp.where(head_a, e, 0.0), axis=1, keepdims=True)
                sb = jnp.sum(jnp.where(head_a, 0.0, e), axis=1, keepdims=True)
                pr = e / jnp.where(head_a, sa, sb)
                return jnp.dot(pr, two(v), preferred_element_type=F32)

            acc = None
            nxt = proj(0)
            o_prev = None
            for p in range(17):
                cur = nxt
                if p + 1 < 16:
                    nxt = proj(p + 1)
                if o_prev is not None:
                    t = jnp.dot(o_prev, wob[(p - 1) * 384:p * 384, :], preferred_element_type=F32)
                    acc = t if acc is None else acc + t
                if p < 16:
                    o_prev = attn(*cur)
            mem[...] = acc[:M]
            xs[r, :] += acc[M:]
            return 0
        jax.lax.fori_loop(0, S // SEG, step, 0)

    def block(i, _):
        layer_a()

        @pl.when(i == 0)
        def _():
            for c in cps:
                c.wait()
        layer_b()
        return 0
    jax.lax.fori_loop(0, 2, block, 0)
    o_ref[...] = xs[...].astype(o_ref.dtype)


@jax.jit
def pallas_interleave_layers__linear_kernel_hedgehog__memory_aug_recurrent_mem_tr__prompt_kernel(
        A_x, A_wqkv, A_w_phi, A_wo, B_x, B_mem0, B_Wq, B_Wk, B_Wv, B_Wo, B_seg_len=None):
    vm = pl.BlockSpec(memory_space=pltpu.VMEM)
    hb = pl.BlockSpec(memory_space=pl.ANY)
    wp = jnp.pad(A_w_phi.reshape(D, 20), ((0, 0), (0, 108)))
    out = pl.pallas_call(
        _kernel,
        out_shape=jax.ShapeDtypeStruct((S, D), A_x.dtype),
        in_specs=[vm] * 5 + [hb] * 4,
        out_specs=vm,
        scratch_shapes=[
            pltpu.VMEM((S, D), F32), pltpu.VMEM((S, D), F32),
            pltpu.VMEM((D, D), BF), pltpu.VMEM((D, D), BF),
            pltpu.VMEM((4, 320, 256), F32), pltpu.VMEM((4, 320, 1), F32),
            pltpu.VMEM((D, HD), BF), pltpu.VMEM((D, HD), BF), pltpu.VMEM((D, HD), BF),
            pltpu.VMEM((HD, D), BF), pltpu.VMEM((M, D), F32),
            pltpu.SemaphoreType.DMA((4,)),
        ],
        compiler_params=pltpu.CompilerParams(vmem_limit_bytes=110 << 20),
    )(A_x.reshape(S, D), A_wqkv, wp, A_wo, B_mem0.reshape(M, D),
      B_Wq.reshape(D, HD), B_Wk.reshape(D, HD), B_Wv.reshape(D, HD), B_Wo.reshape(HD, D))
    return out.reshape(1, S, D)
```

```python
import jax
import jax.numpy as jnp
import jax.experimental.pallas as pl
import jax.experimental.pallas.tpu as pltpu

S, D = 2048, 640
T = 1024
SEG, M, L = 32, 8, 40
HD = 6144
F32, BF = jnp.float32, jnp.bfloat16
NT = (((1,), (1,)), ((), ()))
TN = (((0,), (0,)), ((), ()))
WIN = (0, 128, 256, 384)


def _ln(x):
    m = jnp.mean(x, axis=-1, keepdims=True)
    c = x - m
    v = jnp.mean(c * c, axis=-1, keepdims=True)
    return c * jax.lax.rsqrt(v + 1e-5)


def _iota(shape, d):
    return jax.lax.broadcasted_iota(jnp.int32, shape, d)


def _tdot(a, w, r0, c0, nk, nn):
    outs = [None] * nn
    for k in range(nk):
        for n in range(nn):
            t = jnp.dot(a[:, k * 128:(k + 1) * 128],
                        w[r0 + k * 128:r0 + (k + 1) * 128, c0 + n * 128:c0 + (n + 1) * 128],
                        preferred_element_type=F32)
            outs[n] = t if k == 0 else outs[n] + t
    return jnp.concatenate(outs, axis=1)


def _phi(p):
    p = p.reshape(20, 8, p.shape[-1])
    a = jnp.exp(p - jnp.max(p, axis=0, keepdims=True))
    b = jnp.exp(jnp.min(p, axis=0, keepdims=True) - p)
    a = a / jnp.sum(a, axis=0, keepdims=True)
    b = b / jnp.sum(b, axis=0, keepdims=True)
    return a, b


def _kernel(x_ref, wqkv_ref, wp_ref, wo_ref, mem0_ref, wq_h, wk_h, wv_h, wob_h,
            o_ref, xs, lnb, wqt, wkt, kv, zs, wq, wk, wv, wob, mem, sq, sk, sv, sems):
    cps = [pltpu.make_async_copy(s, d, sems.at[i]) for i, (s, d) in
           enumerate(((wq_h, sq), (wk_h, sk), (wv_h, sv), (wob_h, wob)))]
    for c in cps:
        c.start()

    sel = (_iota((128, D), 0) == (_iota((128, D), 1) % 160) // 8).astype(BF)
    bd = jnp.dot(wp_ref[...], sel, preferred_element_type=F32)
    col = _iota((D, D), 1)
    bd = jnp.where(_iota((D, D), 0) // 20 == (col // 160) * 8 + col % 8, bd, 0.0).astype(BF)
    wqt[...] = jnp.dot(wqkv_ref[:, 0:D], bd, preferred_element_type=F32).T.astype(BF)
    wkt[...] = jnp.dot(wqkv_ref[:, D:2 * D], bd, preferred_element_type=F32).T.astype(BF)
    xs[...] = x_ref[...].astype(F32)

    def layer_a():
        kv[...] = jnp.zeros(kv.shape, F32)
        zs[...] = jnp.zeros(zs.shape, F32)

        def pass1(c, _):
            r = pl.ds(pl.multiple_of(c * T, T), T)
            ln = _ln(xs[r, :])
            lnb[r, :] = ln
            ln = ln.astype(BF)
            v = jnp.dot(ln, wqkv_ref[:, 2 * D:3 * D], preferred_element_type=F32).astype(BF)
            for g in range(4):
                p = jax.lax.dot_general(wkt[g * 160:(g + 1) * 160, :], ln, NT,
                                        preferred_element_type=F32)
                a, b = _phi(p)
                ph = jnp.concatenate([a, b], axis=0).reshape(320, T)
                zs[g] += jnp.sum(ph, axis=1, keepdims=True)
                kv[g] += jnp.dot(ph.astype(BF), v[:, WIN[g]:WIN[g] + 256],
                                 preferred_element_type=F32)
            return 0
        jax.lax.fori_loop(0, S // T, pass1, 0)
        for g in range(4):
            own = (_iota((320, 256), 1) + WIN[g]) // 20 == g * 8 + _iota((320, 256), 0) % 8
            kv[g] = jnp.where(own, kv[g], 0.0)

        def pass2(c, _):
            r = pl.ds(pl.multiple_of(c * T, T), T)
            ln = lnb[r, :].astype(BF)
            os = []
            for g in range(4):
                p = jax.lax.dot_general(wqt[g * 160:(g + 1) * 160, :], ln, NT,
                                        preferred_element_type=F32)
                a, b = _phi(p)
                ph = jnp.concatenate([a, b], axis=0)
                den = jnp.sum(ph * zs[g].reshape(40, 8, 1), axis=0, keepdims=True) + 1e-6
                ph = (ph / den).reshape(320, T).astype(BF)
                os.append(jax.lax.dot_general(ph, kv[g].astype(BF), TN,
                                              preferred_element_type=F32))
            o = jnp.concatenate([os[0][:, :128], os[0][:, 128:] + os[1][:, :128],
                                 os[1][:, 128:] + os[2][:, :128],
                                 os[2][:, 128:] + os[3][:, :128], os[3][:, 128:]], axis=1)
            xs[r, :] += jnp.dot(o.astype(BF), wo_ref[...], preferred_element_type=F32)
            return 0
        jax.lax.fori_loop(0, S // T, pass2, 0)

    def layer_b():
        def lnc(c, _):
            r = pl.ds(pl.multiple_of(c * T, T), T)
            lnb[r, :] = _ln(xs[r, :])
            return 0
        jax.lax.fori_loop(0, S // T, lnc, 0)
        mem[...] = mem0_ref[...].astype(F32)

        def step(s, _):
            r = pl.ds(pl.multiple_of(s * SEG, SEG), SEG)
            h = jnp.concatenate([mem[...], lnb[r, :]], axis=0)
            row = _iota((L, 128), 0)
            lane = _iota((L, 128), 1)
            key = lane % 64
            vis = (row < M) | (row >= key)
            head_a = lane < 64
            real = key < L
            first = _iota((L, 384), 1) < 192
            pad = jnp.zeros((64 - L, 384), F32)

            def two(t):
                return jnp.concatenate([jnp.where(first, t, 0.0), pad,
                                        jnp.where(first, 0.0, t), pad], axis=0).astype(BF)

            def proj(p):
                return [_tdot(h, w, 0, p * 384, 5, 3) for w in (wq, wk, wv)]

            def score(q, k):
                return jax.lax.dot_general(q, two(k), NT, preferred_element_type=F32) * (192 ** -0.5)
            def soft(sc):
                sc = jnp.where(vis, sc, -1000000000.0)
                ninf = -jnp.inf
                ma = jnp.max(jnp.where(head_a & real, sc, ninf), axis=1, keepdims=True)
                mb = jnp.max(jnp.where(head_a | ~real, ninf, sc), axis=1, keepdims=True)
                e = jnp.where(real, jnp.exp(sc - jnp.where(head_a, ma, mb)), 0.0)
                sa = jnp.sum(jnp.where(head_a, e, 0.0), axis=1, keepdims=True)
                sb = jnp.sum(jnp.where(head_a, 0.0, e), axis=1, keepdims=True)
                pr = e / jnp.where(head_a, sa, sb)
                return pr

            acc = None
            qkv, pr, o = {}, {}, {}
            for p in range(19):
                if 0 <= p - 2 < 16:
                    o[p - 2] = jnp.dot(pr[p - 2], two(qkv[p - 2][2]), preferred_element_type=F32)
                if 0 <= p - 1 < 16:
                    pr[p - 1] = soft(score(*qkv[p - 1][:2]))
                if p < 16:
                    qkv[p] = proj(p)
                if 0 <= p - 3:
                    t = _tdot(o[p - 3], wob, (p - 3) * 384, 0, 3, 5)
                    acc = t if acc is None else acc + t
            mem[...] = acc[:M]
            xs[r, :] += acc[M:]
            return 0
        jax.lax.fori_loop(0, S // SEG, step, 0)

    def block(i, _):
        layer_a()

        @pl.when(i == 0)
        def _():
            for c in cps:
                c.wait()

            def flip(p, _):
                r = pl.ds(pl.multiple_of(p * 384, 128), 384)
                for src, dst in ((sq, wq), (sk, wk), (sv, wv)):
                    dst[:, r] = src[r, :].T
                return 0
            jax.lax.fori_loop(0, 16, flip, 0)
        layer_b()
        return 0
    jax.lax.fori_loop(0, 2, block, 0)
    o_ref[...] = xs[...].astype(o_ref.dtype)


@jax.jit
def pallas_interleave_layers__linear_kernel_hedgehog__memory_aug_recurrent_mem_tr__prompt_kernel(
        A_x, A_wqkv, A_w_phi, A_wo, B_x, B_mem0, B_Wq, B_Wk, B_Wv, B_Wo, B_seg_len=None):
    vm = pl.BlockSpec(memory_space=pltpu.VMEM)
    hb = pl.BlockSpec(memory_space=pl.ANY)
    wp = jnp.pad(A_w_phi.reshape(D, 20), ((0, 0), (0, 108)))
    out = pl.pallas_call(
        _kernel,
        out_shape=jax.ShapeDtypeStruct((S, D), A_x.dtype),
        in_specs=[vm] * 5 + [hb] * 4,
        out_specs=vm,
        scratch_shapes=[
            pltpu.VMEM((S, D), F32), pltpu.VMEM((S, D), F32),
            pltpu.VMEM((D, D), BF), pltpu.VMEM((D, D), BF),
            pltpu.VMEM((4, 320, 256), F32), pltpu.VMEM((4, 320, 1), F32),
            pltpu.VMEM((D, HD), BF), pltpu.VMEM((D, HD), BF), pltpu.VMEM((D, HD), BF),
            pltpu.VMEM((HD, D), BF), pltpu.VMEM((M, D), F32),
            *[pltpu.VMEM((HD, D), BF)] * 3,
            pltpu.SemaphoreType.DMA((4,)),
        ],
        compiler_params=pltpu.CompilerParams(vmem_limit_bytes=110 << 20),
    )(A_x.reshape(S, D), A_wqkv, wp, A_wo, B_mem0.reshape(M, D),
      B_Wq.transpose(1, 2, 0).reshape(HD, D), B_Wk.transpose(1, 2, 0).reshape(HD, D), B_Wv.transpose(1, 2, 0).reshape(HD, D), B_Wo.reshape(HD, D))
    return out.reshape(1, S, D)
```

```python
import jax
import jax.numpy as jnp
import jax.experimental.pallas as pl
import jax.experimental.pallas.tpu as pltpu

S, D = 2048, 640
T = 512
OC = 256
SEG, M, L = 32, 8, 40
HD = 6144
F32, BF = jnp.float32, jnp.bfloat16
NT = (((1,), (1,)), ((), ()))
TN = (((0,), (0,)), ((), ()))
WIN = (0, 128, 256, 384)


def _ln(x):
    m = jnp.mean(x, axis=-1, keepdims=True)
    c = x - m
    v = jnp.mean(c * c, axis=-1, keepdims=True)
    return c * jax.lax.rsqrt(v + 1e-5)


def _iota(shape, d):
    return jax.lax.broadcasted_iota(jnp.int32, shape, d)


def _tdot(a, w, r0, c0, nk, nn):
    outs = [None] * nn
    for k in range(nk):
        for n in range(nn):
            t = jnp.dot(a[:, k * 128:(k + 1) * 128],
                        w[r0 + k * 128:r0 + (k + 1) * 128, c0 + n * 128:c0 + (n + 1) * 128],
                        preferred_element_type=F32)
            outs[n] = t if k == 0 else outs[n] + t
    return jnp.concatenate(outs, axis=1)


def _phi(p):
    p = p.reshape(20, 8, p.shape[-1])
    a = jnp.exp(p - jnp.max(p, axis=0, keepdims=True))
    b = jnp.exp(jnp.min(p, axis=0, keepdims=True) - p)
    a = a / jnp.sum(a, axis=0, keepdims=True)
    b = b / jnp.sum(b, axis=0, keepdims=True)
    return a, b


def _kernel(x_h, wqkv_h, wp_h, wo_h, mem0_h, wq_h, wk_h, wv_h, wob_h, o_h,
            xb, wqkv_ref, wp_ref, wo_ref, mem0_ref, xs, lnb, wqt, wkt, wvt, kv, zs,
            wq, wk, wv, wob, mem, sq, sk, sv, sem_a, sem_x, sem_w, sem_o):
    NC = S // T
    WC = HD // NC
    flips = ((wq_h, sq, wq), (wk_h, sk, wk), (wv_h, sv, wv))

    def rows(c, n):
        return pl.ds(pl.multiple_of(c * n, n), n)

    def x_copy(c):
        return pltpu.make_async_copy(x_h.at[rows(c, T)], xb.at[rows(c, T)], sem_x.at[c])

    def w_copy(j, c):
        return pltpu.make_async_copy(flips[j][0].at[rows(c, WC)], flips[j][1].at[rows(c, WC)],
                                     sem_w.at[j, c])

    def o_copy(c):
        return pltpu.make_async_copy(xb.at[rows(c, OC)], o_h.at[rows(c, OC)], sem_o.at[c])

    small = [pltpu.make_async_copy(s_, d_, sem_a.at[i]) for i, (s_, d_) in enumerate(
        ((wp_h, wp_ref), (wqkv_h, wqkv_ref), (wo_h, wo_ref), (mem0_h, mem0_ref), (wob_h, wob)))]
    small[0].start()
    small[1].start()
    for c in range(NC):
        x_copy(c).start()
    small[2].start()
    small[3].start()

    small[0].wait()
    sel = (_iota((160, 128), 1) == _iota((160, 128), 0) // 8).astype(BF)
    bd = jax.lax.dot_general(sel, wp_ref[...], NT, preferred_element_type=F32)
    small[1].wait()
    for c in range(NC):
        for j in range(3):
            w_copy(j, c).start()
    for g in range(4):
        own = (_iota((160, 256), 1) + WIN[g]) // 20 == g * 8 + _iota((160, 256), 0) % 8
        bg = jnp.where(own, bd[:, WIN[g]:WIN[g] + 256], 0.0).astype(BF)
        for t, dst in enumerate((wqt, wkt)):
            w = wqkv_ref[:, t * D + WIN[g]:t * D + WIN[g] + 256]
            dst[g * 160:(g + 1) * 160, :] = jax.lax.dot_general(
                bg, w, NT, preferred_element_type=F32).astype(BF)
    wvt[...] = wqkv_ref[:, 2 * D:3 * D].T

    def layer_a(first):
        kv[...] = jnp.zeros(kv.shape, F32)
        zs[...] = jnp.zeros(zs.shape, F32)

        def proj(w, g, ln):
            return jax.lax.dot_general(w[g * 160:(g + 1) * 160, :], ln, NT, preferred_element_type=F32)

        def pass1(c, _):
            r = rows(c, T)
            if first:
                x_copy(c).wait()
                x = xb[r, :].astype(F32)
                xs[r, :] = x
            else:
                x = xs[r, :]
            ln = _ln(x)
            lnb[r, :] = ln
            ln = ln.astype(BF)
            vt = jax.lax.dot_general(wvt[...], ln, NT, preferred_element_type=F32).astype(BF)
            pk = jax.lax.dot_general(wkt[...], ln, NT, preferred_element_type=F32)
            for g in range(4):
                a, b = _phi(pk[g * 160:(g + 1) * 160])
                ph = jnp.concatenate([a, b], axis=0).reshape(320, T)
                zs[g] += jnp.sum(ph, axis=1, keepdims=True)
                kv[g] += jax.lax.dot_general(vt[g * 160:(g + 1) * 160], ph.astype(BF), NT,
                                             preferred_element_type=F32)
            return 0
        jax.lax.fori_loop(0, NC, pass1, 0)
        own = _iota((160, 320), 0) // 20 == _iota((160, 320), 1) % 8
        for g in range(4):
            kv[g] = jnp.where(own, kv[g], 0.0)
        if first:
            small[2].wait()
            small[4].start()

        def pass2(c, _):
            r = rows(c, T)
            if first:
                for j in range(3):
                    w_copy(j, c).wait()
                for p in range(WC // 384):
                    rr = pl.ds(pl.multiple_of(c * WC + p * 384, 128), 384)
                    for _, src, dst in flips:
                        dst[:, rr] = src[rr, :].T
            ln = lnb[r, :].astype(BF)
            pq = jax.lax.dot_general(wqt[...], ln, NT, preferred_element_type=F32)
            os = []
            for g in range(4):
                a, b = _phi(pq[g * 160:(g + 1) * 160])
                ph = jnp.concatenate([a, b], axis=0)
                den = jnp.sum(ph * zs[g].reshape(40, 8, 1), axis=0, keepdims=True) + 1e-6
                ph = (ph / den).reshape(320, T).astype(BF)
                os.append(jnp.dot(kv[g].astype(BF), ph, preferred_element_type=F32).astype(BF))
            ot = jnp.concatenate(os, axis=0)
            x = xs[r, :] + jax.lax.dot_general(ot, wo_ref[...], TN, preferred_element_type=F32)
            xs[r, :] = x
            lnb[r, :] = _ln(x)
            return 0
        jax.lax.fori_loop(0, NC, pass2, 0)

    def layer_b(i):
        mem[...] = mem0_ref[...].astype(F32)

        def step(s, _):
            r = pl.ds(pl.multiple_of(s * SEG, SEG), SEG)
            h = jnp.concatenate([mem[...], lnb[r, :]], axis=0)
            row = _iota((L, 128), 0)
            lane = _iota((L, 128), 1)
            key = lane % 64
            vis = (row < M) | (row >= key)
            head_a = lane < 64
            real = key < L
            first = _iota((L, 384), 1) < 192
            pad = jnp.zeros((64 - L, 384), F32)

            def two(t):
                return jnp.concatenate([jnp.where(first, t, 0.0), pad,
                                        jnp.where(first, 0.0, t), pad], axis=0).astype(BF)

            def proj(p):
                return [_tdot(h, w, 0, p * 384, 5, 3) for w in (wq, wk, wv)]

            def score(q, k):
                return jax.lax.dot_general(q, two(k), NT, preferred_element_type=F32) * (192 ** -0.5)
            def soft(sc):
                sc = jnp.where(vis, sc, -1000000000.0)
                ninf = -jnp.inf
                ma = jnp.max(jnp.where(head_a & real, sc, ninf), axis=1, keepdims=True)
                mb = jnp.max(jnp.where(head_a | ~real, ninf, sc), axis=1, keepdims=True)
                e = jnp.where(real, jnp.exp(sc - jnp.where(head_a, ma, mb)), 0.0)
                sa = jnp.sum(jnp.where(head_a, e, 0.0), axis=1, keepdims=True)
                sb = jnp.sum(jnp.where(head_a, 0.0, e), axis=1, keepdims=True)
                pr = e / jnp.where(head_a, sa, sb)
                return pr

            acc = None
            qkv, pr, o = {}, {}, {}
            for p in range(19):
                if 0 <= p - 2 < 16:
                    o[p - 2] = jnp.dot(pr[p - 2], two(qkv[p - 2][2]), preferred_element_type=F32)
                if 0 <= p - 1 < 16:
                    pr[p - 1] = soft(score(*qkv[p - 1][:2]))
                if p < 16:
                    qkv[p] = proj(p)
                for j in {16: (9, 10, 11), 17: (12, 13), 18: (14, 15)}.get(p, (p - 7,) if p >= 7 else ()):
                    t = _tdot(o[j], wob, j * 384, 0, 3, 5)
                    acc = t if acc is None else acc + t
            mem[...] = acc[:M]
            xs[r, :] += acc[M:]
            return 0

        def quarter(c, _):
            jax.lax.fori_loop(c * (OC // SEG), (c + 1) * (OC // SEG), step, 0)

            @pl.when(i == 1)
            def _():
                xb[rows(c, OC), :] = xs[rows(c, OC), :].astype(BF)
                o_copy(c).start()
            return 0
        jax.lax.fori_loop(0, S // OC, quarter, 0)

    def block(i, _):
        @pl.when(i == 0)
        def _():
            layer_a(True)
            small[3].wait()
            small[4].wait()

        @pl.when(i == 1)
        def _():
            layer_a(False)
        layer_b(i)
        return 0
    jax.lax.fori_loop(0, 2, block, 0)
    for c in range(S // OC):
        o_copy(c).wait()


@jax.jit
def pallas_interleave_layers__linear_kernel_hedgehog__memory_aug_recurrent_mem_tr__prompt_kernel(
        A_x, A_wqkv, A_w_phi, A_wo, B_x, B_mem0, B_Wq, B_Wk, B_Wv, B_Wo, B_seg_len=None):
    hb = pl.BlockSpec(memory_space=pl.ANY)
    wp = jnp.pad(A_w_phi.reshape(D, 20), ((0, 0), (0, 108)))
    out = pl.pallas_call(
        _kernel,
        out_shape=jax.ShapeDtypeStruct((S, D), A_x.dtype),
        in_specs=[hb] * 9,
        out_specs=hb,
        scratch_shapes=[
            pltpu.VMEM((S, D), BF), pltpu.VMEM((D, 3 * D), BF), pltpu.VMEM((D, 128), BF),
            pltpu.VMEM((D, D), BF), pltpu.VMEM((M, D), BF),
            pltpu.VMEM((S, D), F32), pltpu.VMEM((S, D), F32),
            pltpu.VMEM((D, D), BF), pltpu.VMEM((D, D), BF), pltpu.VMEM((D, D), BF),
            pltpu.VMEM((4, 160, 320), F32), pltpu.VMEM((4, 320, 1), F32),
            pltpu.VMEM((D, HD), BF), pltpu.VMEM((D, HD), BF), pltpu.VMEM((D, HD), BF),
            pltpu.VMEM((HD, D), BF), pltpu.VMEM((M, D), F32),
            *[pltpu.VMEM((HD, D), BF)] * 3,
            pltpu.SemaphoreType.DMA((5,)), pltpu.SemaphoreType.DMA((S // T,)),
            pltpu.SemaphoreType.DMA((3, S // T)), pltpu.SemaphoreType.DMA((S // OC,)),
        ],
        compiler_params=pltpu.CompilerParams(vmem_limit_bytes=110 << 20),
    )(A_x.reshape(S, D), A_wqkv, wp, A_wo, B_mem0.reshape(M, D),
      B_Wq.transpose(1, 2, 0).reshape(HD, D), B_Wk.transpose(1, 2, 0).reshape(HD, D), B_Wv.transpose(1, 2, 0).reshape(HD, D), B_Wo.reshape(HD, D))
    return out.reshape(1, S, D)
```
